```python
import os as _os
_os.environ.setdefault("JAX_PLATFORMS", "cpu")
import jax
import jax.numpy as jnp

def _softmax(x, axis=-1):
    return jax.nn.softmax(x, axis=axis)
def _gelu(x):
    return jax.nn.gelu(x, approximate=True)
def _silu(x):
    return jax.nn.silu(x)
def _sigmoid(x):
    return jax.nn.sigmoid(x)
def _layernorm(x, axis=-1, eps=1e-5):
    m = jnp.mean(x, axis=axis, keepdims=True)
    v = jnp.var(x, axis=axis, keepdims=True)
    return (x - m) / jnp.sqrt(v + eps)
def _scatter_add(tgt, idx, src, axis=0):
    return tgt.at[idx].add(src)
def _segment_sum(src, seg, n):
    return jax.ops.segment_sum(src, seg, n)
class _Rng:
    def __init__(self, key):
        self._k = key
    def _next(self):
        self._k, sub = jax.random.split(self._k)
        return sub
    def normal(self, shape):
        return jax.random.normal(self._next(), shape, dtype=jnp.bfloat16)
    def randint(self, lo, hi, shape):
        return jax.random.randint(self._next(), shape, lo, hi, dtype=jnp.int32)
    def uniform(self, shape, lo=0.0, hi=1.0):
        return jax.random.uniform(self._next(), shape, jnp.bfloat16, lo, hi)
    def permutation(self, n):
        return jax.random.permutation(self._next(), n)


kernel_name = 'interleave_layers__gqa_block_cached__dense_activation_silu__decode'

def setup_inputs():
    _rng = _Rng(jax.random.key(int.from_bytes(__import__("os").urandom(4), "little")))
    _w = (lambda a: (lambda t: t.astype(jnp.bfloat16) if jnp.issubdtype(t.dtype, jnp.floating) else t)(jnp.asarray(a)))
    def _A_setup():
        B, Sq, D = 2, 1, 512
        Hq, Hkv, Sk, Dh = 32, 8, 8192, 128
        assert Hq % Hkv == 0, (Hq, Hkv)
        return {
            "x": _w((lambda *s: _rng.normal(s) * 0.1)(B, Sq, D)),
            "k_cache": _w((lambda *s: _rng.normal(s) * 0.8)(B, Hkv, Sk, Dh)),
            "v_cache": _w((lambda *s: _rng.normal(s) * 1.6)(B, Hkv, Sk, Dh)),
            "wq": _w((lambda *s: _rng.normal(s) * 0.8)(D, Hq * Dh) * (D ** -0.5)),
            "wo": _w((lambda *s: _rng.normal(s) * 1.6)(Hq * Dh, D) * ((Hq * Dh) ** -0.5)),
        }
    _A_in = _A_setup()

    def _B_setup():
        B, S, D, F = 2, 1, 512, 1792
        return {
            "x": _w((lambda *s: _rng.normal(s) * 0.1)(B, S, D)),
            "w1": _w((lambda *s: _rng.normal(s) * 0.4)(D, F) * (D ** -0.5)),
            "w2": _w((lambda *s: _rng.normal(s) * 0.4)(F, D) * (F ** -0.5)),
        }
    _B_in = _B_setup()

    return {
        "A_x": _A_in["x"],
        "A_k_cache": _A_in["k_cache"],
        "A_v_cache": _A_in["v_cache"],
        "A_wq": _A_in["wq"],
        "A_wo": _A_in["wo"],
        "B_x": _B_in["x"],
        "B_w1": _B_in["w1"],
        "B_w2": _B_in["w2"],
    }

def reference(A_x, A_k_cache, A_v_cache, A_wq, A_wo, B_x, B_w1, B_w2):
    def _A_ref(x, k_cache, v_cache, wq, wo):
        B, Sq, D = x.shape
        Hq, Dh = 32, 128
        Hkv = k_cache.shape[1]
        rep = Hq // Hkv
        q = (lambda x, *d: x.transpose(*d))((x @ wq).reshape(B, Sq, Hq, Dh), 0, 2, 1, 3)
        k = jnp.repeat(k_cache, rep, axis=1)
        v = jnp.repeat(v_cache, rep, axis=1)
        scores = jnp.einsum("bhqd,bhkd->bhqk", q, k) * (Dh ** -0.5)
        p = _softmax(scores, axis=-1)
        o = jnp.einsum("bhqk,bhkd->bhqd", p, v)
        return (lambda x, *d: x.transpose(*d))(o, 0, 2, 1, 3).reshape(B, Sq, Hq * Dh) @ wo

    def _B_ref(x, w1, w2):
        h = jnp.einsum("bsd,df->bsf", x, w1)
        h = _silu(h)
        out = jnp.einsum("bsf,fd->bsd", h, w2)
        return out

    x = A_x
    x = x + _A_ref(_layernorm(x, axis=-1), A_k_cache, A_v_cache, A_wq, A_wo)
    x = x + _B_ref(_layernorm(x, axis=-1), B_w1, B_w2)
    x = x + _A_ref(_layernorm(x, axis=-1), A_k_cache, A_v_cache, A_wq, A_wo)
    x = x + _B_ref(_layernorm(x, axis=-1), B_w1, B_w2)
    return x
```

```python
import jax
import jax.numpy as jnp
from jax import lax
import jax.experimental.pallas as pl
import jax.experimental.pallas.tpu as pltpu

B, D, HKV, REP, SK, DH, F = 2, 512, 8, 4, 8192, 128, 1792
H = SK // 2
TB = 2048
VSPLIT = 4
PS = SK // VSPLIT
f32, bf16, u32 = jnp.float32, jnp.bfloat16, jnp.uint32


def _dot(a, b):
    return jnp.dot(a, b, preferred_element_type=f32)


def _asb(t):
    return pltpu.bitcast(t, bf16)


def _kernel(x_hbm, k_hbm, v_hbm, wq_hbm, wo_hbm, w1_hbm, w2_hbm, o_ref,
            xs, kv, vv, wqv, wov, w1v, w2v, kt, wq2, wo2, w12, w22,
            qs, ps, ls, cq, c1, outs, sems, vsems):
    row = lax.broadcasted_iota(jnp.int32, (8, DH), 0)

    cx = pltpu.make_async_copy(x_hbm, xs, sems.at[0])
    cw = [pltpu.make_async_copy(s, d, sems.at[1 + i]) for i, (s, d) in enumerate(
        ((wq_hbm, wqv), (wo_hbm, wov), (w1_hbm, w1v), (w2_hbm, w2v)))]

    def kcopy(b, h):
        return pltpu.make_async_copy(k_hbm.at[b, h], kv.at[b, h], sems.at[5 + b * 16 + h])

    def vcopy(b, h):
        return pltpu.make_async_copy(v_hbm.at[b, h], vv.at[b, h], sems.at[13 + b * 16 + h])

    def vlast(i):
        r = pl.ds(i * PS, PS)
        return pltpu.make_async_copy(v_hbm.at[B - 1, HKV - 1, r], vv.at[B - 1, HKV - 1, r], vsems.at[i])

    cx.start()
    for c in cw:
        c.start()
    for b in range(B):
        for h in range(HKV):
            kcopy(b, h).start()
        for h in range(HKV - (b == B - 1)):
            vcopy(b, h).start()
    for i in range(VSPLIT):
        vlast(i).start()
    cx.wait()

    def relayout(c, src, dst, step):
        c.wait()

        def body(i, carry):
            r = pl.ds(pl.multiple_of(i * step, step), step)
            r2 = pl.ds(pl.multiple_of(i * (step // 2), step // 2), step // 2)
            dst[r2, :] = pltpu.bitcast(src[r, :], u32)
            return carry
        lax.fori_loop(0, src.shape[0] // step, body, 0)

    relayout(cw[0], wqv, wq2, 16)
    relayout(cw[1], wov, wo2, 128)
    relayout(cw[2], w1v, w12, 32)
    relayout(cw[3], w2v, w22, 128)
    vv32 = vv.bitcast(u32)

    ones = jnp.ones((8, D), bf16)
    cq[...] = _dot(ones, _asb(wq2[...]))
    c1[...] = _dot(ones, _asb(w12[...]))

    def ln_matmul(xb, w, c):
        xr = xb.astype(bf16)
        y = _dot(xr, _asb(w[...]))
        xf = xr.astype(f32)
        m = jnp.mean(xf, axis=-1, keepdims=True)
        d = xf - m
        r = lax.rsqrt(jnp.mean(d * d, axis=-1, keepdims=True) + 1e-5)
        return (y - m * c[...]) * r

    def qproj(xb):
        qf = ln_matmul(xb, wq2, cq)
        for h in range(HKV):
            o = h * REP * DH
            q = qf[:, o:o + DH]
            for j in range(1, REP):
                q = jnp.where(row % REP == j, qf[:, o + j * DH:o + (j + 1) * DH], q)
            qs[h] = q

    def qk(h):
        q = qs[h]
        qa = jnp.where(row < REP, q, 0.).astype(bf16)
        qb = jnp.where(row >= REP, q, 0.).astype(bf16)
        return _dot(qa, _asb(kt[h, :, :H])) + _dot(qb, _asb(kt[h, :, H:]))

    def softmax(s):
        s = s * (DH ** -0.5)
        m = jnp.max(s, axis=-1, keepdims=True)
        m = jnp.maximum(m, pltpu.roll(m, REP, 0))
        p = jnp.exp(s - m)
        l = jnp.sum(p, axis=-1, keepdims=True)
        return p, 1.0 / (l + pltpu.roll(l, REP, 0))

    def pv(b, h, p, inv_l, last=False):
        r2 = lax.broadcasted_iota(jnp.int32, p.shape, 0)
        pa = jnp.where(r2 < REP, p, 0.).astype(bf16)
        pb = jnp.where(r2 >= REP, p, 0.).astype(bf16)
        if last:
            o = None
            for i in range(VSPLIT):
                if i == 0:
                    pl.when(b < B - 1)(vcopy(0, HKV - 1).wait)
                pl.when(b == B - 1)(vlast(i).wait)
                pp = pa if i < VSPLIT // 2 else pb
                c0 = (i * PS) % H
                t = _dot(pp[:, c0:c0 + PS], _asb(vv32[b, h, i * PS // 2:(i + 1) * PS // 2]))
                o = t if o is None else o + t
        else:
            o = _dot(pa, _asb(vv32[b, h, :H // 2])) + _dot(pb, _asb(vv32[b, h, H // 2:]))
        o = (o + pltpu.roll(o, REP, 0)) * inv_l
        return jnp.concatenate([jnp.where(row == j, o, 0.) for j in range(REP)], axis=1).astype(bf16)

    def ffn(xb):
        hh = ln_matmul(xb, w12, c1)
        hh = hh * jax.nn.sigmoid(hh)
        return _dot(hh.astype(bf16), _asb(w22[...]))

    def rowsum(acc):
        return jnp.broadcast_to(jnp.sum(acc, axis=0, keepdims=True), (8, D))

    x0 = xs[...].astype(f32)

    def batch(b, carry):
        xb = jnp.broadcast_to(jnp.where(b == 0, x0[0:1], x0[1:2]), (8, D))

        qproj(xb)

        def kbody(h, c):
            kcopy(b, h).wait()

            def tbody(i, c2):
                r = pl.ds(pl.multiple_of(i * TB, TB), TB)
                kt[h, :, r] = pltpu.bitcast(kv[b, h, r, :].T, u32)
                return c2
            lax.fori_loop(0, SK // TB, tbody, 0)
            p, inv_l = softmax(qk(h))
            ps[h] = p
            ls[h] = jnp.broadcast_to(inv_l, (8, DH))
            return c
        lax.fori_loop(0, HKV, kbody, 0)

        n = REP * DH // 2

        def vbody(h, acc):
            vcopy(b, h).wait()
            w = wo2[pl.ds(pl.multiple_of(h * n, n), n), :]
            return acc + _dot(pv(b, h, ps[h], ls[h]), _asb(w))
        acc = lax.fori_loop(0, HKV - 1, vbody, jnp.zeros((8, D), f32))
        o7 = pv(b, HKV - 1, ps[HKV - 1], ls[HKV - 1], True)
        acc = acc + _dot(o7, _asb(wo2[(HKV - 1) * n:, :]))
        xb = xb + rowsum(acc)
        xb = xb + ffn(xb)

        qproj(xb)
        s = qk(0)
        heads = []
        for h in range(HKV):
            p, inv_l = softmax(s)
            if h + 1 < HKV:
                s = qk(h + 1)
            heads.append(pv(b, h, p, inv_l))
        xb = xb + rowsum(_dot(jnp.concatenate(heads, axis=1), _asb(wo2[...])))
        xb = xb + ffn(xb)
        outs[b] = xb
        return carry
    lax.fori_loop(0, B, batch, 0)
    o_ref[...] = jnp.concatenate([outs[0][0:1], outs[1][0:1]], axis=0).astype(bf16)


@jax.jit
def pallas_interleave_layers__gqa_block_cached__dense_activation_silu__decode_kernel(
    A_x: jax.Array,
    A_k_cache: jax.Array,
    A_v_cache: jax.Array,
    A_wq: jax.Array,
    A_wo: jax.Array,
    B_x: jax.Array,
    B_w1: jax.Array,
    B_w2: jax.Array,
):
    del B_x
    vm = pltpu.VMEM
    big = (A_k_cache, A_v_cache, A_wq, A_wo, B_w1, B_w2)
    scratch = (
        [vm((B, D), bf16)]
        + [vm(a.shape, a.dtype) for a in big]
        + [vm((HKV, DH // 2, SK), u32)]
        + [vm((w.shape[0] // 2, w.shape[1]), u32) for w in big[2:]]
        + [vm((HKV, 8, DH), f32), vm((HKV, 8, H), f32), vm((HKV, 8, DH), f32),
           vm((8, HKV * REP * DH), f32), vm((8, F), f32), vm((B, 8, D), f32),
           pltpu.SemaphoreType.DMA((37,)), pltpu.SemaphoreType.DMA((VSPLIT,))]
    )
    out = pl.pallas_call(
        _kernel,
        out_shape=jax.ShapeDtypeStruct((B, D), bf16),
        in_specs=[pl.BlockSpec(memory_space=pl.ANY)] * 7,
        out_specs=pl.BlockSpec(memory_space=pltpu.VMEM),
        scratch_shapes=scratch,
        compiler_params=pltpu.CompilerParams(vmem_limit_bytes=116 * 2**20),
    )(A_x.reshape(B, D), *big)
    return out.reshape(B, 1, D)
```
